```python
import jax
import jax.numpy as jnp

def _softmax(x, axis=-1):
    return jax.nn.softmax(x, axis=axis)
def _gelu(x):
    return jax.nn.gelu(x, approximate=True)
def _silu(x):
    return jax.nn.silu(x)
def _sigmoid(x):
    return jax.nn.sigmoid(x)
def _layernorm(x, axis=-1, eps=1e-5):
    m = jnp.mean(x, axis=axis, keepdims=True)
    v = jnp.var(x, axis=axis, keepdims=True)
    return (x - m) / jnp.sqrt(v + eps)
def _scatter_add(tgt, idx, src, axis=0):
    return tgt.at[idx].add(src)
def _segment_sum(src, seg, n):
    return jax.ops.segment_sum(src, seg, n)
class _Rng:
    def __init__(self, key):
        self._k = key
    def _next(self):
        self._k, sub = jax.random.split(self._k)
        return sub
    def normal(self, shape):
        return jax.random.normal(self._next(), shape, dtype=jnp.bfloat16)
    def randint(self, lo, hi, shape):
        return jax.random.randint(self._next(), shape, lo, hi, dtype=jnp.int32)
    def uniform(self, shape, lo=0.0, hi=1.0):
        return jax.random.uniform(self._next(), shape, jnp.bfloat16, lo, hi)
    def permutation(self, n):
        return jax.random.permutation(self._next(), n)


kernel_name = 'standalone__layernorm_linear__prompt'

def setup_inputs():
    _rng = _Rng(jax.random.key(int.from_bytes(__import__("os").urandom(4), "little")))
    _w = (lambda a: (lambda t: t.astype(jnp.bfloat16) if jnp.issubdtype(t.dtype, jnp.floating) else t)(jnp.asarray(a)))
    B, S, D = 2, 2048, 1024
    return {
        "x": _w((lambda *s: _rng.normal(s) * 0.05)(B, S, D)),
        "g": _w((lambda *s: _rng.normal(s) * 0.05)(D) + 1.0),
        "b": _w((lambda *s: _rng.normal(s) * 0.05)(D)),
        "w": _w((lambda *s: _rng.normal(s) * 0.05)(D, D)),
    }

def reference(x, g, b, w):
    return (_layernorm(x, axis=-1) * g + b) @ w
```

```python
import jax
import jax.numpy as jnp
import jax.experimental.pallas as pl
import jax.experimental.pallas.tpu as pltpu

_EPS = 1e-5


def _ln_linear_kernel(x_ref, g_ref, b_ref, w_ref, o_ref):
    x = x_ref[...].astype(jnp.float32)
    m = jnp.mean(x, axis=-1, keepdims=True)
    xc = x - m
    v = jnp.mean(xc * xc, axis=-1, keepdims=True)
    y = xc * jax.lax.rsqrt(v + _EPS)
    y = y * g_ref[...].astype(jnp.float32) + b_ref[...].astype(jnp.float32)
    o_ref[...] = jnp.dot(
        y.astype(jnp.bfloat16), w_ref[...], preferred_element_type=jnp.float32
    ).astype(o_ref.dtype)


@jax.jit
def pallas_standalone__layernorm_linear__prompt_kernel(
    x: jax.Array,
    g: jax.Array,
    b: jax.Array,
    w: jax.Array,
):
    B, S, D = x.shape
    N = w.shape[1]
    M = B * S
    bm = 512
    x2 = x.reshape(M, D)
    g2 = g.reshape(1, D)
    b2 = b.reshape(1, D)
    out = pl.pallas_call(
        _ln_linear_kernel,
        grid=(M // bm,),
        in_specs=[
            pl.BlockSpec((bm, D), lambda i: (i, 0)),
            pl.BlockSpec((1, D), lambda i: (0, 0)),
            pl.BlockSpec((1, D), lambda i: (0, 0)),
            pl.BlockSpec((D, N), lambda i: (0, 0)),
        ],
        out_specs=pl.BlockSpec((bm, N), lambda i: (i, 0)),
        out_shape=jax.ShapeDtypeStruct((M, N), x.dtype),
        compiler_params=pltpu.CompilerParams(
            dimension_semantics=("arbitrary",),
            vmem_limit_bytes=64 * 1024 * 1024,
        ),
    )(x2, g2, b2, w)
    return out.reshape(B, S, N)
```

```python
import functools

import jax
import jax.numpy as jnp
import jax.experimental.pallas as pl
import jax.experimental.pallas.tpu as pltpu

_EPS = 1e-5

_SIZES = (320, 128, 256, 512, 1024, 1856)
_W_CHUNKS = (256, 256, 256, 256)
_TAIL_ROWS = (512, 512, 576, 256)
_TAIL_COLS = (512, 256, 256)
_LN_ROWS = 128


def _layernorm_rows(x_ref, g, b, y_ref, r0, rows):
    x = x_ref[pl.ds(r0, rows), :].astype(jnp.float32)
    inv_d = 1.0 / x.shape[-1]
    m = jnp.sum(x, axis=-1, keepdims=True) * inv_d
    xc = x - m
    v = jnp.sum(xc * xc, axis=-1, keepdims=True) * inv_d
    y = xc * jax.lax.rsqrt(v + _EPS)
    y = y * g + b
    y_ref[pl.ds(r0, rows), :] = y.astype(y_ref.dtype)


def _kernel(*refs, n_out):
    nb = len(_SIZES)
    nw = len(_W_CHUNKS)
    x_hbm, g_hbm, b_hbm, w_hbm, o_hbm = refs[:5]
    rest = refs[5:]
    xs, ys, os_ = rest[:nb], rest[nb:2 * nb], rest[2 * nb:3 * nb]
    w_buf, g_buf, b_buf, sx, so, sw, sg, sbar = rest[3 * nb:]
    starts = [sum(_SIZES[:i]) for i in range(nb)]
    cstarts = [sum(_W_CHUNKS[:i]) for i in range(nw)]

    def x_copy(i):
        return pltpu.make_async_copy(
            x_hbm.at[pl.ds(starts[i], _SIZES[i]), :], xs[i], sx.at[i])

    def w_copy(c):
        cs = pl.ds(cstarts[c], _W_CHUNKS[c])
        return pltpu.make_async_copy(w_hbm.at[:, cs], w_buf.at[:, cs], sw.at[c])

    g_copy = pltpu.make_async_copy(g_hbm, g_buf, sg.at[0])
    b_copy = pltpu.make_async_copy(b_hbm, b_buf, sg.at[1])

    def fence():
        pl.semaphore_signal(sbar, 1)
        pl.semaphore_wait(sbar, 1)

    out_copies = []

    def out_start(i, r0, rows, c0, cols):
        rs, cs = pl.ds(r0, rows), pl.ds(c0, cols)
        c = pltpu.make_async_copy(
            os_[i].at[rs, cs],
            o_hbm.at[pl.ds(starts[i] + r0, rows), cs],
            so.at[len(out_copies)])
        c.start(priority=1)
        out_copies.append(c)

    def matmul(i, r0, rows, c0, cols):
        os_[i][pl.ds(r0, rows), pl.ds(c0, cols)] = jnp.dot(
            ys[i][pl.ds(r0, rows), :], w_buf[:, pl.ds(c0, cols)],
            preferred_element_type=jnp.float32).astype(os_[i].dtype)

    queue = [x_copy(0), g_copy, b_copy, w_copy(0), w_copy(1), w_copy(2),
             x_copy(1), w_copy(3)] + [x_copy(i) for i in range(2, nb)]
    for c in queue:
        c.start()
        fence()

    x_copy(0).wait()
    g_copy.wait()
    b_copy.wait()
    g = g_buf[...].astype(jnp.float32).reshape(1, -1)
    b = b_buf[...].astype(jnp.float32).reshape(1, -1)

    def layernorm(i):
        for r0 in range(0, _SIZES[i], _LN_ROWS):
            _layernorm_rows(xs[i], g, b, ys[i], r0, min(_LN_ROWS, _SIZES[i] - r0))

    layernorm(0)
    for c in range(nw):
        w_copy(c).wait()
        if c == nw - 1:
            x_copy(1).wait()
        matmul(0, 0, _SIZES[0], cstarts[c], _W_CHUNKS[c])
        if c == nw - 1:
            layernorm(1)

    for h in range(1, nb - 1):
        x_copy(h + 1).wait()
        if h == nb - 2:
            for i in range(h):
                out_start(i, 0, _SIZES[i], 0, n_out)
        matmul(h, 0, _SIZES[h], 0, n_out)
        if h == nb - 2:
            out_start(h, 0, _SIZES[h], 0, n_out)
        layernorm(h + 1)

    fence()
    last = nb - 1
    r0 = 0
    for rows in _TAIL_ROWS[:-1]:
        matmul(last, r0, rows, 0, n_out)
        out_start(last, r0, rows, 0, n_out)
        r0 += rows
    c0 = 0
    for cols in _TAIL_COLS:
        matmul(last, r0, _TAIL_ROWS[-1], c0, cols)
        out_start(last, r0, _TAIL_ROWS[-1], c0, cols)
        c0 += cols

    for c in out_copies:
        c.wait()


@jax.jit
def pallas_standalone__layernorm_linear__prompt_kernel(
    x: jax.Array,
    g: jax.Array,
    b: jax.Array,
    w: jax.Array,
):
    B, S, D = x.shape
    N = w.shape[1]
    M = B * S
    assert sum(_SIZES) == M and sum(_W_CHUNKS) == N
    assert sum(_TAIL_ROWS) == _SIZES[-1] and sum(_TAIL_COLS) == N
    n_out_dmas = len(_SIZES) - 1 + len(_TAIL_ROWS) - 1 + len(_TAIL_COLS)
    out = pl.pallas_call(
        functools.partial(_kernel, n_out=N),
        in_specs=[pl.BlockSpec(memory_space=pl.ANY)] * 4,
        out_specs=pl.BlockSpec(memory_space=pl.ANY),
        out_shape=jax.ShapeDtypeStruct((M, N), x.dtype),
        scratch_shapes=(
            [pltpu.VMEM((s, D), x.dtype) for s in _SIZES]
            + [pltpu.VMEM((s, D), jnp.bfloat16) for s in _SIZES]
            + [pltpu.VMEM((s, N), x.dtype) for s in _SIZES]
            + [pltpu.VMEM((D, N), w.dtype),
               pltpu.VMEM((D,), g.dtype),
               pltpu.VMEM((D,), b.dtype),
               pltpu.SemaphoreType.DMA((len(_SIZES),)),
               pltpu.SemaphoreType.DMA((n_out_dmas,)),
               pltpu.SemaphoreType.DMA((len(_W_CHUNKS),)),
               pltpu.SemaphoreType.DMA((2,)),
               pltpu.SemaphoreType.REGULAR]),
        compiler_params=pltpu.CompilerParams(
            vmem_limit_bytes=64 * 1024 * 1024,
            flags={"XLA_TPU_EVENLY_DISTRIBUTE_CRITICAL_NODES": True},
        ),
    )(x.reshape(M, D), g, b, w)
    return out.reshape(B, S, N)
```

```python
import functools

import jax
import jax.numpy as jnp
import jax.experimental.pallas as pl
import jax.experimental.pallas.tpu as pltpu

_EPS = 1e-5

_SIZES = (272, 128, 256, 512, 1024, 1904)
_K_CHUNK = 256
_K_FIRST = 256
_TAIL_ROWS = (1024, 624, 128, 128)
_TAIL_COLS = (512, 256, 256)
_LN_ROWS = 128


def _layernorm_rows(x_ref, g, b, y_ref, r0, rows):
    x = x_ref[pl.ds(r0, rows), :].astype(jnp.float32)
    inv_d = 1.0 / x.shape[-1]
    m = jnp.sum(x, axis=-1, keepdims=True) * inv_d
    xc = x - m
    v = jnp.sum(xc * xc, axis=-1, keepdims=True) * inv_d
    y = xc * jax.lax.rsqrt(v + _EPS)
    y = y * g + b
    y_ref[pl.ds(r0, rows), :] = y.astype(y_ref.dtype)


def _kernel(*refs):
    nb = len(_SIZES)
    x_hbm, g_hbm, b_hbm, w_hbm, o_hbm = refs[:5]
    rest = refs[5:]
    xs, ys, os_ = rest[:nb], rest[nb:2 * nb], rest[2 * nb:3 * nb]
    w_buf, g_buf, b_buf, acc, sx, so, sw, sg, sbar = rest[3 * nb:]
    d_in, n_out = w_hbm.shape
    nk = d_in // _K_CHUNK
    starts = [sum(_SIZES[:i]) for i in range(nb)]

    def x_copy(i):
        return pltpu.make_async_copy(
            x_hbm.at[pl.ds(starts[i], _SIZES[i]), :], xs[i], sx.at[i])

    def w_copy(c):
        ks = pl.ds(c * _K_CHUNK, _K_CHUNK)
        return pltpu.make_async_copy(w_hbm.at[ks, :], w_buf.at[ks, :], sw.at[c])

    g_copy = pltpu.make_async_copy(g_hbm, g_buf, sg.at[0])
    b_copy = pltpu.make_async_copy(b_hbm, b_buf, sg.at[1])

    def fence():
        pl.semaphore_signal(sbar, 1)
        pl.semaphore_wait(sbar, 1)

    out_copies = []

    def out_start(i, r0, rows, c0, cols):
        cs = pl.ds(c0, cols)
        c = pltpu.make_async_copy(
            os_[i].at[pl.ds(r0, rows), cs],
            o_hbm.at[pl.ds(starts[i] + r0, rows), cs],
            so.at[len(out_copies)])
        c.start(priority=1)
        out_copies.append(c)

    def matmul(i, r0, rows, c0, cols):
        os_[i][pl.ds(r0, rows), pl.ds(c0, cols)] = jnp.dot(
            ys[i][pl.ds(r0, rows), :], w_buf[:, pl.ds(c0, cols)],
            preferred_element_type=jnp.float32).astype(os_[i].dtype)

    def matmul_k_chunk(i, r0, rows, c):
        ks = pl.ds(c * _K_CHUNK, _K_CHUNK)
        a = acc.at[pl.ds(0, rows), :]
        p = jnp.dot(ys[i][pl.ds(r0, rows), ks], w_buf[ks, :],
                    preferred_element_type=jnp.float32)
        if c == 0:
            a[...] = p
        elif c < nk - 1:
            a[...] = a[...] + p
        else:
            os_[i][pl.ds(r0, rows), :] = (a[...] + p).astype(os_[i].dtype)

    def matmul_rows(i, r0, rows):
        lead = min(_K_FIRST, rows)
        for c in range(nk):
            matmul_k_chunk(i, r0, lead, c)
        if lead < rows:
            matmul(i, r0 + lead, rows - lead, 0, n_out)

    queue = ([x_copy(0), g_copy, b_copy] + [w_copy(c) for c in range(nk - 1)]
             + [x_copy(1), w_copy(nk - 1)] + [x_copy(i) for i in range(2, nb)])
    for c in queue:
        c.start()
        fence()

    x_copy(0).wait()
    g_copy.wait()
    b_copy.wait()
    g = g_buf[...].astype(jnp.float32).reshape(1, -1)
    b = b_buf[...].astype(jnp.float32).reshape(1, -1)

    def layernorm(i):
        for r0 in range(0, _SIZES[i], _LN_ROWS):
            _layernorm_rows(xs[i], g, b, ys[i], r0, min(_LN_ROWS, _SIZES[i] - r0))

    layernorm(0)
    for c in range(nk):
        w_copy(c).wait()
        if c == nk - 1:
            x_copy(1).wait()
        matmul_k_chunk(0, 0, _SIZES[0], c)
        if c == nk - 1:
            layernorm(1)

    for h in range(1, nb - 1):
        x_copy(h + 1).wait()
        if h == nb - 2:
            for i in range(h):
                out_start(i, 0, _SIZES[i], 0, n_out)
        matmul_rows(h, 0, _SIZES[h])
        if h == nb - 2:
            out_start(h, 0, _SIZES[h], 0, n_out)
        layernorm(h + 1)

    fence()
    last = nb - 1
    r0 = 0
    for t, rows in enumerate(_TAIL_ROWS[:-1]):
        if t == 0:
            matmul_rows(last, r0, rows)
        else:
            matmul(last, r0, rows, 0, n_out)
        out_start(last, r0, rows, 0, n_out)
        r0 += rows
    c0 = 0
    for cols in _TAIL_COLS:
        matmul(last, r0, _TAIL_ROWS[-1], c0, cols)
        out_start(last, r0, _TAIL_ROWS[-1], c0, cols)
        c0 += cols

    for c in out_copies:
        c.wait()


@jax.jit
def pallas_standalone__layernorm_linear__prompt_kernel(
    x: jax.Array,
    g: jax.Array,
    b: jax.Array,
    w: jax.Array,
):
    B, S, D = x.shape
    N = w.shape[1]
    M = B * S
    assert sum(_SIZES) == M and D % _K_CHUNK == 0
    assert sum(_TAIL_ROWS) == _SIZES[-1] and sum(_TAIL_COLS) == N
    n_out_dmas = len(_SIZES) - 1 + len(_TAIL_ROWS) - 1 + len(_TAIL_COLS)
    acc_rows = max(_SIZES[0], _K_FIRST)
    out = pl.pallas_call(
        _kernel,
        in_specs=[pl.BlockSpec(memory_space=pl.ANY)] * 4,
        out_specs=pl.BlockSpec(memory_space=pl.ANY),
        out_shape=jax.ShapeDtypeStruct((M, N), x.dtype),
        scratch_shapes=(
            [pltpu.VMEM((s, D), x.dtype) for s in _SIZES]
            + [pltpu.VMEM((s, D), jnp.bfloat16) for s in _SIZES]
            + [pltpu.VMEM((s, N), x.dtype) for s in _SIZES]
            + [pltpu.VMEM((D, N), w.dtype),
               pltpu.VMEM((D,), g.dtype),
               pltpu.VMEM((D,), b.dtype),
               pltpu.VMEM((acc_rows, N), jnp.float32),
               pltpu.SemaphoreType.DMA((len(_SIZES),)),
               pltpu.SemaphoreType.DMA((n_out_dmas,)),
               pltpu.SemaphoreType.DMA((D // _K_CHUNK,)),
               pltpu.SemaphoreType.DMA((2,)),
               pltpu.SemaphoreType.REGULAR]),
        compiler_params=pltpu.CompilerParams(
            vmem_limit_bytes=64 * 1024 * 1024,
            flags={"XLA_TPU_EVENLY_DISTRIBUTE_CRITICAL_NODES": True},
        ),
    )(x.reshape(M, D), g, b, w)
    return out.reshape(B, S, N)
```
